```python
import jax
import jax.numpy as jnp

def _softmax(x, axis=-1):
    return jax.nn.softmax(x, axis=axis)
def _gelu(x):
    return jax.nn.gelu(x, approximate=True)
def _silu(x):
    return jax.nn.silu(x)
def _sigmoid(x):
    return jax.nn.sigmoid(x)
def _layernorm(x, axis=-1, eps=1e-5):
    m = jnp.mean(x, axis=axis, keepdims=True)
    v = jnp.var(x, axis=axis, keepdims=True)
    return (x - m) / jnp.sqrt(v + eps)
def _scatter_add(tgt, idx, src, axis=0):
    return tgt.at[idx].add(src)
def _segment_sum(src, seg, n):
    return jax.ops.segment_sum(src, seg, n)
class _Rng:
    def __init__(self, key):
        self._k = key
    def _next(self):
        self._k, sub = jax.random.split(self._k)
        return sub
    def normal(self, shape):
        return jax.random.normal(self._next(), shape, dtype=jnp.bfloat16)
    def randint(self, lo, hi, shape):
        return jax.random.randint(self._next(), shape, lo, hi, dtype=jnp.int32)
    def uniform(self, shape, lo=0.0, hi=1.0):
        return jax.random.uniform(self._next(), shape, jnp.bfloat16, lo, hi)
    def permutation(self, n):
        return jax.random.permutation(self._next(), n)


kernel_name = 'recurrent_scan__linear_kernel_hedgehog__dense_activation_relu__prompt'

def _fwd_setup_inputs():
    _rng = _Rng(jax.random.key(int.from_bytes(__import__("os").urandom(4), "little")))
    _w = (lambda a: (lambda t: t.astype(jnp.bfloat16) if jnp.issubdtype(t.dtype, jnp.floating) else t)(jnp.asarray(a)))
    def _A_setup():
        B, S, D, H = 1, 2048, 1024, 32
        Dh = D // H
        return {
            "x": _w((lambda *s: _rng.normal(s) * 0.05)(B, S, D)),
            "wqkv": _w((lambda *s: _rng.normal(s) * 0.05)(D, 3 * D)),
            "w_phi": _w((lambda *s: _rng.normal(s) * 0.05)(H, Dh, Dh) * (Dh ** -0.5)),
            "wo": _w((lambda *s: _rng.normal(s) * 0.05)(D, D)),
        }
    _A_in = _A_setup()

    def _B_setup():
        B, S, D, Dff = 1, 2048, 1024, 3584
        return {
            "x": _w((lambda *s: _rng.normal(s) * 0.05)(B, S, D)),
            "w1": _w((lambda *s: _rng.normal(s) * 0.05)(D, Dff)),
            "w2": _w((lambda *s: _rng.normal(s) * 0.05)(Dff, D)),
        }
    _B_in = _B_setup()

    return {
        "A_x": _A_in["x"],
        "A_wqkv": _A_in["wqkv"],
        "A_w_phi": _A_in["w_phi"],
        "A_wo": _A_in["wo"],
        "B_x": _B_in["x"],
        "B_w1": _B_in["w1"],
        "B_w2": _B_in["w2"],
    }

def _fwd_reference(A_x, A_wqkv, A_w_phi, A_wo, B_x, B_w1, B_w2):
    def _A_ref(x, wqkv, w_phi, wo):
        B, S, D = x.shape
        H = 32; Dh = D // H
        qkv = (lambda x, *d: x.transpose(*d))((x @ wqkv).reshape(B, S, 3, H, Dh), 2, 0, 3, 1, 4)
        q, k, v = qkv[0], qkv[1], qkv[2]
        pq = jnp.einsum("bhsd,hdf->bhsf", q, w_phi)
        pk = jnp.einsum("bhsd,hdf->bhsf", k, w_phi)
        phi_q = jnp.concatenate([_softmax(pq, axis=-1), _softmax(-pq, axis=-1)], axis=-1)
        phi_k = jnp.concatenate([_softmax(pk, axis=-1), _softmax(-pk, axis=-1)], axis=-1)
        kv = jnp.einsum("bhsf,bhsd->bhfd", phi_k, v)
        z  = jnp.einsum("bhsf->bhf", phi_k)
        num = jnp.einsum("bhqf,bhfd->bhqd", phi_q, kv)
        den = jnp.einsum("bhqf,bhf->bhq", phi_q, z)[..., None] + 1e-6
        o = num / den
        return (lambda x, *d: x.transpose(*d))(o, 0, 2, 1, 3).reshape(B, S, D) @ wo

    def _B_ref(x, w1, w2):
        h = jnp.einsum("bsd,df->bsf", x, w1)
        zero = jnp.zeros_like(h)
        h = jnp.maximum(h, zero)
        return jnp.einsum("bsf,fd->bsd", h, w2)

    x = A_x
    xn = _layernorm(x, axis=-1)
    s = _A_ref(xn, A_wqkv, A_w_phi, A_wo)
    g = _silu(_B_ref(xn, B_w1, B_w2))
    return x + s * g


def setup_inputs():
    _inp = _fwd_setup_inputs()
    _gk = jax.random.fold_in(jax.random.key(int.from_bytes(__import__("os").urandom(4), "little")), 2**31 - 1)
    _shapes = [[1, 2048, 1024]]
    _dtypes = ['bfloat16']
    _gks = jax.random.split(_gk, len(_shapes))
    _gs = [jax.random.normal(k, s, dtype=jnp.dtype(d)) * 0.05 for k, s, d in zip(_gks, _shapes, _dtypes)]
    _inp["grad_out"] = _gs[0]
    return _inp

def reference(A_x, A_wqkv, A_w_phi, A_wo, B_w1, B_w2, B_x, grad_out):
    _const = dict(B_x=B_x)
    def _f(*_d):
        return _fwd_reference(**{'A_x': _d[0], 'A_wqkv': _d[1], 'A_w_phi': _d[2], 'A_wo': _d[3], 'B_w1': _d[4], 'B_w2': _d[5], **_const})
    _out, _vjp = jax.vjp(_f, A_x, A_wqkv, A_w_phi, A_wo, B_w1, B_w2)
    _grads = _vjp(grad_out)
    _out0 = jnp.asarray(_out)
    return (_out0, *[jnp.asarray(_g) for _g in _grads])
```

```python
import jax
import jax.numpy as jnp
from jax import lax
import jax.experimental.pallas as pl
import jax.experimental.pallas.tpu as pltpu

S, D, H, DH, F = 2048, 1024, 32, 32, 3584
T = 512
NT = S // T
TH = T // 2
C = 512
NC = F // C
NQ = 3 * D // C
G = D // 128
BF, F32 = jnp.bfloat16, jnp.float32


def _nn(a, b):
    return lax.dot_general(a, b, (((1,), (0,)), ((), ())), preferred_element_type=F32)


def _nt(a, b):
    return lax.dot_general(a, b, (((1,), (1,)), ((), ())), preferred_element_type=F32)


def _tn(a, b):
    return lax.dot_general(a, b, (((0,), (0,)), ((), ())), preferred_element_type=F32)


def _layer_norm(x):
    d = x - jnp.mean(x, axis=-1, keepdims=True)
    rstd = lax.rsqrt(jnp.mean(d * d, axis=-1, keepdims=True) + 1e-5)
    return d * rstd, rstd


def _heads(v):
    return v.reshape(v.shape[0] // DH, DH, v.shape[1])


def _dual_softmax(p):
    p3 = _heads(p)
    ep = jnp.exp(p3 - jnp.max(p3, axis=1, keepdims=True))
    em = jnp.exp(jnp.min(p3, axis=1, keepdims=True) - p3)
    sp = ep * (1.0 / jnp.sum(ep, axis=1, keepdims=True))
    sm = em * (1.0 / jnp.sum(em, axis=1, keepdims=True))
    return jnp.concatenate([sp.reshape(p.shape), sm.reshape(p.shape)], axis=0)


def _dual_softmax_bwd(phi, dphi):
    t = _heads(phi * dphi)
    u = (t - _heads(phi) * jnp.sum(t, axis=1, keepdims=True)).reshape(phi.shape)
    return u[:128] - u[128:]


def _pair(phi, p):
    return jnp.concatenate([phi[p * 64:(p + 1) * 64], phi[128 + p * 64:128 + (p + 1) * 64]], axis=0)


def _apply(kvt, phi):
    return jnp.concatenate([_nn(kvt[p * 64:(p + 1) * 64], _pair(phi, p)) for p in range(2)], axis=0)


def _outer(v, phi):
    return jnp.concatenate([_nt(v[p * 64:(p + 1) * 64], _pair(phi, p)) for p in range(2)], axis=0)


def _fold(v):
    r = v[:, :128]
    for j in range(1, v.shape[1] // 128):
        r = r + v[:, j * 128:(j + 1) * 128]
    return r


def _lanes(v, n):
    return jnp.concatenate([v] * (n // 128), axis=1)


_U = ((1, 0, 0, 1), (0, 0, 1, 1), (1, 0, 0, 0), (0, 0, 0, 1), (1, 1, 0, 0), (-1, 0, 1, 0), (0, 1, 0, -1))
_V = ((1, 0, 0, 1), (1, 0, 0, 0), (0, 1, 0, -1), (-1, 0, 1, 0), (0, 0, 0, 1), (1, 1, 0, 0), (0, 0, 1, 1))
_W = ((1, 0, 0, 1), (0, 0, 1, -1), (0, 1, 0, 1), (1, 0, 1, 0), (-1, 1, 0, 0), (0, 0, 0, 1), (1, 0, 0, 0))


_H_ORDER, _F_ORDER = (1, 0, 3, 4, 6, 2, 5), (2, 4, 5, 3, 1, 0, 6)
_DX_ORDER, _DW_ORDER = (6, 5, 0, 1, 4, 2, 3), (6, 5, 0, 3, 2, 1, 4)
_DA_ORDER, _DW2_ORDER = (1, 4, 0, 5, 6, 2, 3), (2, 3, 0, 5, 6, 1, 4)


def _signed_sum(terms):
    first = [sgn for sgn, _ in terms].index(1)
    r = terms[first][1]
    for sgn, t in terms[:first] + terms[first + 1:]:
        r = r + t if sgn > 0 else r - t
    return r


def _quads(top, bot):
    n = top.shape[1] // 2
    return [top[:, :n], top[:, n:], bot[:, :n], bot[:, n:]]


def _operands(m, quads):
    ops = []
    for row in m:
        terms = [(sgn, q) for sgn, q in zip(row, quads) if sgn]
        if len(terms) > 1:
            terms = [(sgn, q.astype(F32)) for sgn, q in terms]
        ops.append(_signed_sum(terms).astype(BF))
    return ops


def _sum_f32(row, pair):
    return jnp.concatenate([_signed_sum([(sgn, q.astype(F32)) for sgn, q in zip(row, qs) if sgn])
                            for qs in pair], axis=1)


def _quads4(v):
    return _quads(v[:v.shape[0] // 2], v[v.shape[0] // 2:])


def _join(q):
    return jnp.concatenate([jnp.concatenate(q[:2], axis=1), jnp.concatenate(q[2:], axis=1)], axis=0)


def _combine(m, prods):
    return [_signed_sum([(m[r][j], p) for r, p in prods.items() if m[r][j]]) for j in range(4)]


def _strassen(m, order, dot, lhs, rhs, filler=None):
    prods = {}
    for r in order:
        prods[r] = dot(lhs[r], rhs[r])
        if filler is not None:
            next(filler, None)
    return _combine(m, prods)


def _bits(v):
    return lax.bitcast_convert_type(v.astype(F32), jnp.int32)


def _token(deps, zero):
    tok = None
    for d in deps:
        d = _bits(d)
        for a in range(0, d.shape[0], 16):
            for b in range(0, d.shape[1], 128):
                t = d[a:a + 8, b:b + 128]
                tok = t if tok is None else tok | t
    return jnp.concatenate([tok & zero] * 2, axis=0)


def _after(v, pieces, zero):
    kb = min(v.shape[0], 512)
    nb = 128 * (512 // kb)
    pieces, cols = list(pieces), []
    for n in range(0, v.shape[1], nb):
        col = []
        for k in range(0, v.shape[0], kb):
            t = v[k:k + kb, n:n + nb]
            if pieces:
                head = lax.bitcast_convert_type(_bits(t[:16, :128]) | _token(pieces.pop(0), zero), F32).astype(BF)
                if nb > 128:
                    head = jnp.concatenate([head, t[:16, 128:]], axis=1)
                t = jnp.concatenate([head, t[16:]], axis=0)
            col.append(t)
        cols.append(jnp.concatenate(col, axis=0))
    assert not pieces
    return jnp.concatenate(cols, axis=1)


def _split(vs, n):
    return [[v[k * (v.shape[0] // n):(k + 1) * (v.shape[0] // n)] for v in vs] for k in range(n)] if vs else []


def _kernel(x_hbm, wqkv_hbm, wphi_hbm, wo_hbm, w1_hbm, w2_hbm, dy_hbm,
            out_hbm, dx_hbm, dwqkv_hbm, dwphi_hbm, dwo_hbm, dw1_hbm, dw2_hbm,
            x_v, dy_v, wqkv_v, wo_v, w1_v, w2_v, wp_v, ux_v, uxt_v, a_v,
            wos_v, dp_v, dxn_v, dwo_acc, bd_v, kv_acc, z_acc, kvt_v, kvb_v, zb_v, dden_v, zero_v, wphi_v, sems):
    sem_ids = iter(range(96))
    vt_v = wqkv_v
    df_v = ux_v

    def copies(pairs):
        return [pltpu.make_async_copy(s, d, sems.at[next(sem_ids)]) for s, d in pairs]

    def chunk_copies(n, src, dst):
        base = next(sem_ids)
        for _ in range(n - 1):
            next(sem_ids)
        return lambda c: pltpu.make_async_copy(src(c), dst(c), sems.at[base + c])

    def trows(i):
        return pl.ds(pl.multiple_of(i * T, T), T)

    def hrows(i):
        return pl.ds(pl.multiple_of(i * TH, TH), TH)

    def crows(c):
        return pl.ds(pl.multiple_of(c * C, C), C)

    def phik(i, g):
        return dp_v.at[D // C + g // 2, g % 2, hrows(i)]

    def phiq(i, g):
        return dp_v.at[g // 2 + (NQ - 2 if g >= G // 2 else 0), g % 2, hrows(i)]

    def dnum_ref(i, g):
        return dxn_v.at[g // 4, pl.ds(pl.multiple_of(i * TH + (g // 2) % 2 * 128, 128), 128), pl.ds(g % 2 * T, T)]

    x_copy = chunk_copies(NT, lambda i: x_hbm.at[trows(i)], lambda i: x_v.at[trows(i)])
    w1_copy = chunk_copies(NC, lambda c: w1_hbm.at[:, crows(c)], lambda c: w1_v.at[c])
    w2_copy = chunk_copies(NC, lambda c: w2_hbm.at[crows(c)], lambda c: w2_v.at[crows(c)])
    wqkv_copy = chunk_copies(NQ, lambda c: wqkv_hbm.at[:, crows(c)], lambda c: wqkv_v.at[c])
    for i in range(NT):
        x_copy(i).start()
    w1_copy(0).start()
    w2_copy(0).start()
    zero_v[...] = jnp.zeros_like(zero_v)

    def clear(i, _):
        for ref in (dxn_v.at[0], dxn_v.at[1], dwo_acc):
            ref[pl.ds(pl.multiple_of(i * 64, 64), 64), :] = jnp.zeros((64, D), F32)
        return 0

    lax.fori_loop(0, D // 64, clear, 0)

    def p0(i, _):
        x_copy(i).wait()
        for b in range(0, TH, 32):
            top, bot = [_layer_norm(x_v[pl.ds(pl.multiple_of(i * T + j * TH + b, 32), 32), :].astype(F32))[0]
                        for j in range(2)]
            for r, u in enumerate(_operands(_U, _quads(top, bot))):
                ux_v[r, pl.ds(pl.multiple_of(i * TH + b, 32), 32), :] = u
        return 0

    with jax.named_scope("p0"):
        lax.fori_loop(0, NT, p0, 0)
    in_rest = copies([(wo_hbm, wo_v), (dy_hbm, dy_v), (wphi_hbm, wphi_v)])

    def v_w1(c):
        return _operands(_V, _quads(w1_v[c, :D // 2], w1_v[c, D // 2:]))

    def v_w2(c):
        w = w2_v[crows(c), :]
        return _operands(_V, _quads(w[:C // 2], w[C // 2:]))

    def accumulate(quads, rows=slice(None)):
        for j, q in enumerate(quads):
            dxn_v[j // 2, rows, (j % 2) * (D // 2):(j % 2 + 1) * (D // 2)] += q

    def pf(c, _):
        @pl.when(c < NC - 1)
        def _():
            w1_copy(c + 1).start()
            w2_copy(c + 1).start()
            wqkv_copy(c).start()

        @pl.when(c == NC - 1)
        def _():
            for cp in in_rest:
                cp.start()

        w1_copy(c).wait()
        w2_copy(c).wait()
        uxt_v[c] = ux_v[c].T
        hq = _strassen(_W, _H_ORDER, _nn, ux_v, v_w1(c))
        aq = [jnp.where(h < 0.0, -0.0, jnp.abs(h)) for h in hq]
        for j, a in enumerate(aq):
            a_v[c, j] = a.astype(BF)
        accumulate(_strassen(_W, _F_ORDER, _nn, _operands(_U, aq), v_w2(c)))
        return 0

    with jax.named_scope("pf"):
        lax.fori_loop(0, NC, pf, 0)
    for c in range(NQ):
        wqkv_copy(c).wait()
    for cp in in_rest:
        cp.wait()

    ri = lax.broadcasted_iota(jnp.int32, (128, 128), 0)
    ci = lax.broadcasted_iota(jnp.int32, (128, 128), 1)
    blk = (ri // DH) == (ci // DH)
    same_head = (ri // DH) % 2 == (ci // DH) % 2

    bdt = []
    for g in range(G):
        w = wphi_v[g * 128:(g + 1) * 128, :].astype(F32)
        bd = jnp.where(blk, jnp.concatenate([w] * 4, axis=1), 0.0)
        bd_v[g] = bd.astype(BF)
        bdt.append(bd.T.astype(BF))
    for c in range(NQ):
        if c < 2 * D // C:
            wt = jnp.concatenate([_nt(bdt[(c * (C // 128) + j) % G], wqkv_v[c, :, j * 128:(j + 1) * 128])
                                  for j in range(C // 128)], axis=0)
        else:
            wt = wqkv_v[c].T
        q = _quads(wt[:C // 2], wt[C // 2:])
        for r, v in enumerate(_operands(_V, [q[0], q[2], q[1], q[3]])):
            wp_v[c // 2, r, (c % 2) * (C // 2):(c % 2 + 1) * (C // 2), :] = v
    wo_ops, free = [], iter(range(6))
    wo_quads = [wo_v.at[pl.ds((j // 2) * (D // 2), D // 2), pl.ds((j % 2) * (D // 2), D // 2)] for j in range(4)]
    for row, v in zip(_V, _operands(_V, [q[...] for q in wo_quads])):
        if sum(map(abs, row)) == 1:
            wo_ops.append(wo_quads[row.index(1)])
        else:
            k = next(free)
            wo_ops.append(wqkv_v.at[4 + k // 2, pl.ds((k % 2) * (D // 2), D // 2)] if k < 4 else wos_v)
            wo_ops[-1][...] = v
    kv_acc[...] = jnp.zeros_like(kv_acc)
    z_acc[...] = jnp.zeros_like(z_acc)

    def groups(prods):
        q = _combine(_W, prods)
        lo, hi = jnp.concatenate([q[0], q[2]], axis=1), jnp.concatenate([q[1], q[3]], axis=1)
        return [(lo, hi)[(g // 2) % 2][(g // 4) * 256 + (g % 2) * 128:(g // 4) * 256 + (g % 2 + 1) * 128]
                for g in range(G)]

    def gate_parts(i, j):
        tr = pl.ds(pl.multiple_of(i * T + (j // 2) * TH, TH), TH)
        cs = slice((j % 2) * (D // 2), (j % 2 + 1) * (D // 2))
        f = dxn_v[j // 2, hrows(i), cs]
        return f, dy_v[tr, cs].astype(F32), 0.5 * jnp.tanh(0.5 * f) + 0.5, x_v.at[tr, cs]

    def p1(i, _):
        proj = lambda k, r: _nn(wp_v[k, r], uxt_v[r, :, hrows(i)])
        pk = groups({r: proj(1, r) for r in range(7)})
        prods, phis = {}, []
        for g in range(G):
            phi = _dual_softmax(pk[g])
            z_acc[g] += _fold(phi)
            phis.append(phi.astype(BF))
            phik(i, g)[...] = phis[g]
            if g < 7:
                prods[g] = proj(0, g)
        pq, prods = groups(prods), {}
        for g in range(G):
            if g < 7:
                prods[g] = proj(2, g)
            phiq(i, g)[...] = _dual_softmax(pq[g]).astype(BF)
        for g, v in enumerate(groups(prods)):
            v = v.astype(BF)
            vt_v[i, g * 128:(g + 1) * 128, :] = v
            kv_acc[g] += _outer(v, phis[g])
        return 0

    with jax.named_scope("p1"):
        lax.fori_loop(0, NT, p1, 0)

    def finish_state():
        for g in range(G):
            kvt = jnp.where(same_head, kv_acc[g], 0.0)
            kvt_v[g] = kvt.astype(BF)
            kv = kvt.T
            for j in range(2):
                part = kv[j * 64:(j + 1) * 64]
                kvb_v[g, j * 128:(j + 1) * 128, :] = jnp.where(
                    blk, jnp.concatenate([part, part], axis=0), 0.0).astype(BF)
            zb_v[g] = jnp.broadcast_to(jnp.sum(z_acc[g], axis=1, keepdims=True), (256, 128))
        kv_acc[...] = jnp.zeros_like(kv_acc)
        z_acc[...] = jnp.zeros_like(z_acc)

    finish_state()

    def p2(i, _):
        wds = _operands(_W, [dy * (f * sg) for f, dy, sg, _ in (gate_parts(i, j) for j in range(4))])
        os_, rdens, prods = {}, {}, {}
        for g, r in ((0, None), (4, 6), (1, 5), (5, None), (2, 0), (6, None), (3, 3), (7, 1), (None, 4), (None, 2)):
            if r is not None:
                prods[r] = _nt(wo_ops[r][...], wds[r])
            if g is None:
                continue
            pz = phiq(i, g)[...].astype(F32) * _lanes(zb_v[g], T)
            rdens[g] = 1.0 / (jnp.sum(_heads(pz[:128] + pz[128:]), axis=1, keepdims=True) + 1e-6)
            os_[g] = _heads(_apply(kvt_v[g], phiq(i, g)[...])) * rdens[g]
        q = _combine(_U, prods)
        dot = jnp.concatenate([jnp.concatenate([q[0], q[2]], axis=1), jnp.concatenate([q[1], q[3]], axis=1)], axis=0)
        ot = jnp.concatenate([os_[g].reshape(128, T) for g in range(G)], axis=0)
        q = _quads(ot[:D // 2], ot[D // 2:])
        uot = _operands(_U, [q[0], q[2], q[1], q[3]])

        sq = _combine(_W, {r: _nn(uot[r].T, wo_ops[r][...]) for r in _H_ORDER})
        dfs = []
        for j in range(4):
            f, dy, sg, x = gate_parts(i, j)
            x[...] = (x[...].astype(F32) + sq[j] * (f * sg)).astype(BF)
            dfs.append(dy * sq[j] * (sg * (1.0 + f * (1.0 - sg))))
        wdf = _operands(_W, dfs)
        for r in range(7):
            df_v[r, hrows(i), :] = wdf[r]
        for g in range(G):
            dnum = _heads(dot[g * 128:(g + 1) * 128]) * rdens[g]
            dden_v[i, g] = -jnp.sum(dnum * os_[g], axis=1, keepdims=True)
            dnum_ref(i, g)[...] = dnum.reshape(128, T)
        prods = {r: _nn(uot[r], wds[r]) for r in _DW_ORDER}
        for j, q in enumerate(_combine(_V, prods)):
            dwo_acc[(j // 2) * (D // 2):(j // 2 + 1) * (D // 2), (j % 2) * (D // 2):(j % 2 + 1) * (D // 2)] += q
        return 0

    with jax.named_scope("p2"):
        lax.fori_loop(0, NT, p2, 0)
    out_cp = copies([(x_v, out_hbm)])
    for cp in out_cp:
        cp.start()
    wo_v[...] = dwo_acc[...].astype(BF)
    dwo_cp = copies([(wo_v, dwo_hbm)])
    dwo_cp[0].start()

    dw2_copy = chunk_copies(NC, lambda c: w2_v.at[crows(c)], lambda c: dw2_hbm.at[crows(c)])
    dw1_copy = chunk_copies(NC, lambda c: w1_v.at[c], lambda c: dw1_hbm.at[:, crows(c)])
    qkv_copy = chunk_copies(NQ, lambda c: wqkv_v.at[c], lambda c: dwqkv_hbm.at[:, crows(c)])

    def p4(c, _, filler=None):
        aq = [a_v[c, j] for j in range(4)]
        daq = _strassen(_U, _DA_ORDER, _nt, df_v, v_w2(c), filler)
        dw2 = _strassen(_V, _DW2_ORDER, _tn, _operands(_U, aq), df_v, filler)
        for j in range(4):
            bits = _bits(aq[j])
            a_v[c, j] = jnp.where(bits < 0, 0.0, jnp.where(bits == 0, 0.5 * daq[j], daq[j])).astype(BF)
            w2_v[pl.ds(pl.multiple_of(c * C + (j // 2) * (C // 2), C // 2), C // 2),
                 (j % 2) * (D // 2):(j % 2 + 1) * (D // 2)] = dw2[j].astype(BF)
        dw2_copy(c).start()
        return 0

    def q_bwd(i):
        dps = []
        for g in range(G):
            dden = jnp.broadcast_to(dden_v[i, g], (4, DH, T)).reshape(128, T)
            dden = jnp.concatenate([dden, dden], axis=0)
            dnum = dnum_ref(i, g)[...].astype(BF)
            phib = phiq(i, g)[...]
            phi = phib.astype(F32)
            kv_acc[g] += _outer(dnum, phib)
            z_acc[g] += _fold(phi * dden)
            dphi = _nn(kvb_v[g], dnum) + _lanes(zb_v[g], T) * dden
            dps.append(_dual_softmax_bwd(phi, dphi).astype(BF).T)
            yield
            if g < 2:
                yield
        for g in range(G):
            for j in range(2):
                dp_v[g // 4, j, hrows(i), (g % 4) * 128:(g % 4 + 1) * 128] = dps[g][j * TH:(j + 1) * TH]
        for j in range(2):
            dxn_v[j, hrows(i), :] = jnp.zeros((TH, D), F32)

    def p4_q(i, _):
        filler = q_bwd(i)
        p4(i, 0, filler)
        list(filler)
        return 0

    def px_last(n, _):
        rows = pl.ds(pl.multiple_of(n * (S // 4), S // 4), S // 4)
        ws = _operands(_W, [a_v[NC - 1, j, rows, :] for j in range(4)])
        accumulate(_strassen(_U, _DX_ORDER, _nt, ws, v_w1(NC - 1)), rows)
        return 0

    def px2(n, grads, weights, dot, pieces=()):
        k, rows = n // 2, pl.ds(pl.multiple_of(n % 2 * (S // 4), S // 4), S // 4)
        pair, pieces, prods = [grads(2 * k + j, rows) for j in range(2)], list(pieces), {}
        for r in _DX_ORDER:
            vs = _operands(_V, weights(k, r))
            for t in _DX_ORDER[1::2]:
                if pieces and prods:
                    vs[t] = _after(vs[t], [pieces.pop(0)], zero_v[...])
            prods[r] = _join(_strassen(_U, _DX_ORDER, dot, _operands(_W, _quads4(_sum_f32(_W[r], pair))), vs))
        accumulate(_combine(_U, prods), rows)

    def px_ffn2(n, _):
        pair = [_quads4(w1_v[n // 2 * 2 + j]) for j in range(2)]
        px2(n, lambda c, rows: [a_v[c, j, rows, :] for j in range(4)],
            lambda k, r: _quads4(_sum_f32(_V[r], pair)), _nt)
        return 0

    def px_ffn_kv(i, _):
        dps, dvs = [], []
        for g in range(G):
            phib = phik(i, g)[...]
            dphi = _nn(kvb_v[g], vt_v[i, g * 128:(g + 1) * 128, :]) + _lanes(zb_v[g], T)
            dvs.append(_apply(kvt_v[g], phib).astype(BF).T)
            dps.append(_dual_softmax_bwd(phib.astype(F32), dphi).astype(BF).T)
        px_ffn2(i, 0)
        for k, d in enumerate(dps + dvs):
            for j in range(2):
                dp_v[D // C + k // 4, j, hrows(i), (k % 4) * 128:(k % 4 + 1) * 128] = d[j * TH:(j + 1) * TH]
        return 0

    def px_att(n, _):
        def weights(k, r):
            q = _quads4(wp_v[k, r])
            return [q[0], q[2], q[1], q[3]]

        px2(n, lambda c, rows: _quads(dp_v[c, 0, rows, :], dp_v[c, 1, rows, :]), weights, _nn,
            _split(uu_prep(n), 16))
        return 0

    sums = [k for k in range(7) if sum(map(abs, _U[k])) > 1]

    def uu(r, k):
        if k in sums[:4]:
            return ux_v.at[r, pl.ds(sums.index(k) * 256, 256)]
        if k in sums:
            return dp_v.at[NQ + r // 4, r // 2 % 2, pl.ds(pl.multiple_of(r % 2 * 256, 256), 256)]
        j = _U[k].index(1)
        return uxt_v.at[r, pl.ds(j % 2 * 256, 256), pl.ds(j // 2 * 512, 512)]

    def uu_prep(r):
        q = _quads4(uxt_v[r])
        ops = _operands(_U, [q[0], q[2], q[1], q[3]])
        for k in sums:
            uu(r, k)[...] = ops[k]
        return [ops[k] for k in sums]

    def wgrad(quads, pieces=()):
        pieces, prods = list(pieces), {}
        for r in _DW_ORDER:
            w = _sum_f32(_W[r], [quads])
            ws = _operands(_W, _quads4(w))
            for k in _DW_ORDER[1::2]:
                if pieces and prods:
                    ws[k] = _after(ws[k], [pieces.pop(0)], zero_v[...])
            prods[r] = _join(_strassen(_V, _DW_ORDER, _nn, [uu(r, k)[...] for k in range(7)], ws))
        return _join(_combine(_V, prods)).astype(BF)

    def py_ffn_ln(c, _):
        pieces = []
        for k in range(4):
            half, sub = k // 2, k % 2 * (TH // 2)
            tr = pl.ds(pl.multiple_of(c * T + half * TH + sub, TH // 2), TH // 2)
            dxn = dxn_v[half, pl.ds(pl.multiple_of(c * TH + sub, TH // 2), TH // 2), :]
            xn, rstd = _layer_norm(x_v[tr, :].astype(F32))
            m1 = jnp.mean(dxn, axis=-1, keepdims=True)
            m2 = jnp.mean(dxn * xn, axis=-1, keepdims=True)
            dx = (dy_v[tr, :].astype(F32) + rstd * (dxn - m1 - xn * m2)).astype(BF)
            dy_v[tr, :] = dx
            pieces += _split([dx], 4)
        w1_v[c] = wgrad([a_v[c, j] for j in range(4)], pieces)
        dw1_copy(c).start()
        return 0

    def py_qk(c, _):
        gm = wgrad(_quads(dp_v[c, 0], dp_v[c, 1]))
        for j in range(C // 128):
            g = (c * (C // 128) + j) % G
            gj = gm[:, j * 128:(j + 1) * 128]
            kv_acc[g] += _tn(wqkv_v[c, :, j * 128:(j + 1) * 128], gj)
            wqkv_v[c, :, j * 128:(j + 1) * 128] = _nt(gj, bd_v[g]).astype(BF)
        qkv_copy(c).start()
        return 0

    def py_v(c, _):
        wqkv_v[c] = wgrad(_quads(dp_v[c, 0], dp_v[c, 1]))
        qkv_copy(c).start()
        return 0

    def py_ffn(c, _):
        w1_v[c] = wgrad([a_v[c, j] for j in range(4)])
        dw1_copy(c).start()
        return 0

    with jax.named_scope("p4"):
        lax.fori_loop(0, NT, p4_q, 0)
        lax.fori_loop(NT, NC, p4, 0)
        finish_state()
    with jax.named_scope("pxa"):
        lax.fori_loop(0, NT, px_ffn_kv, 0)
    out_cp[0].wait()
    for i in range(NT):
        x_copy(i).start()
        wqkv_copy(i).start()
    with jax.named_scope("pxb"):
        lax.fori_loop(NT, NC - 1, px_ffn2, 0)
        uu_prep(NQ)
        lax.fori_loop(0, 2, px_last, 0)
    with jax.named_scope("pxc"):
        lax.fori_loop(0, NQ, px_att, 0, unroll=2)
    for i in range(NT):
        x_copy(i).wait()
        wqkv_copy(i).wait()
    with jax.named_scope("pyl"):
        lax.fori_loop(0, NT, py_ffn_ln, 0)
    dx_cp = copies([(dy_v, dx_hbm)])
    for cp in dx_cp:
        cp.start()
    with jax.named_scope("pya"):
        lax.fori_loop(0, NT, py_qk, 0)
    for g in range(G):
        for j in range(4):
            wphi_v[g * 128 + j * DH:g * 128 + (j + 1) * DH, :] = (
                kv_acc[g, j * DH:(j + 1) * DH, j * DH:(j + 1) * DH].astype(BF))
    dwphi_cp = copies([(wphi_v, dwphi_hbm)])
    dwphi_cp[0].start()
    with jax.named_scope("pyb"):
        lax.fori_loop(NT, NQ, py_v, 0, unroll=True)
    with jax.named_scope("pyc"):
        lax.fori_loop(NT, NC, py_ffn, 0)
    for cp in dwo_cp + dx_cp + dwphi_cp:
        cp.wait()
    for c in range(NQ):
        qkv_copy(c).wait()
    for c in range(NC):
        dw2_copy(c).wait()
        dw1_copy(c).wait()


@jax.jit
def pallas_recurrent_scan__linear_kernel_hedgehog__dense_activation_relu__prompt_kernel(
    A_x: jax.Array,
    A_wqkv: jax.Array,
    A_w_phi: jax.Array,
    A_wo: jax.Array,
    B_x: jax.Array,
    B_w1: jax.Array,
    B_w2: jax.Array,
    grad_out: jax.Array,
):
    hbm = pl.BlockSpec(memory_space=pl.ANY)
    sds = lambda *s: jax.ShapeDtypeStruct(s, BF)
    V = pltpu.VMEM
    out, dx, dwqkv, dwphi, dwo, dw1, dw2 = pl.pallas_call(
        _kernel,
        in_specs=[hbm] * 7,
        out_specs=[hbm] * 7,
        out_shape=[sds(S, D), sds(S, D), sds(D, 3 * D), sds(H * DH, DH), sds(D, D), sds(D, F), sds(F, D)],
        scratch_shapes=[
            V((S, D), BF), V((S, D), BF), V((NQ, D, C), BF), V((D, D), BF), V((NC, D, C), BF), V((F, D), BF),
            V((3, 7, C, D // 2), BF), V((7, S // 2, D // 2), BF), V((7, D // 2, S // 2), BF),
            V((NC, 4, S // 2, C // 2), BF), V((D // 2, D // 2), BF),
            V((NQ + 2, 2, S // 2, C), BF), V((2, S // 2, D), F32), V((D, D), F32),
            V((G, 128, 128), BF), V((G, 128, 128), F32), V((G, 256, 128), F32), V((G, 128, 128), BF),
            V((G, 256, 128), BF), V((G, 256, 128), F32), V((NT, G, 4, 1, T), F32), V((8, 128), jnp.int32), V((H * DH, DH), BF), pltpu.SemaphoreType.DMA((96,)),
        ],
        compiler_params=pltpu.CompilerParams(vmem_limit_bytes=127 * 1024 * 1024),
    )(A_x.reshape(S, D), A_wqkv, A_w_phi.reshape(H * DH, DH), A_wo, B_w1, B_w2, grad_out.reshape(S, D))
    return (out.reshape(1, S, D), dx.reshape(1, S, D), dwqkv, dwphi.reshape(H, DH, DH), dwo, dw1, dw2)
```
